```python
import os as _os
_os.environ.setdefault("JAX_PLATFORMS", "cpu")
import jax
import jax.numpy as jnp

def _softmax(x, axis=-1):
    return jax.nn.softmax(x, axis=axis)
def _gelu(x):
    return jax.nn.gelu(x, approximate=True)
def _silu(x):
    return jax.nn.silu(x)
def _sigmoid(x):
    return jax.nn.sigmoid(x)
def _layernorm(x, axis=-1, eps=1e-5):
    m = jnp.mean(x, axis=axis, keepdims=True)
    v = jnp.var(x, axis=axis, keepdims=True)
    return (x - m) / jnp.sqrt(v + eps)
def _scatter_add(tgt, idx, src, axis=0):
    return tgt.at[idx].add(src)
def _segment_sum(src, seg, n):
    return jax.ops.segment_sum(src, seg, n)
class _Rng:
    def __init__(self, key):
        self._k = key
    def _next(self):
        self._k, sub = jax.random.split(self._k)
        return sub
    def normal(self, shape):
        return jax.random.normal(self._next(), shape, dtype=jnp.bfloat16)
    def randint(self, lo, hi, shape):
        return jax.random.randint(self._next(), shape, lo, hi, dtype=jnp.int32)
    def uniform(self, shape, lo=0.0, hi=1.0):
        return jax.random.uniform(self._next(), shape, jnp.bfloat16, lo, hi)
    def permutation(self, n):
        return jax.random.permutation(self._next(), n)


kernel_name = 'gated_mix__grouped_kv_mqa__swiglu_ffn__prompt'

def setup_inputs():
    _rng = _Rng(jax.random.key(int.from_bytes(__import__("os").urandom(4), "little")))
    _w = (lambda a: (lambda t: t.astype(jnp.bfloat16) if jnp.issubdtype(t.dtype, jnp.floating) else t)(jnp.asarray(a)))
    def _A_setup():
        B, S, D, H = 1, 2048, 512, 32
        Dh = D // H
        return {
            "x": _w((lambda *s: _rng.normal(s) * 0.05)(B, S, D)),
            "wq": _w((lambda *s: _rng.normal(s) * 0.4)(D, H * Dh)),
            "wk": _w((lambda *s: _rng.normal(s) * 0.4)(D, Dh)),
            "wv": _w((lambda *s: _rng.normal(s) * 0.05)(D, Dh)),
            "wo": _w((lambda *s: _rng.normal(s) * 0.05)(H * Dh, D)),
        }
    _A_in = _A_setup()

    def _B_setup():
        B, S, D, F = 1, 2048, 512, 1792
        return {
            "x": _w((lambda *s: _rng.normal(s) * 0.05)(B, S, D)),
            "w_gate": _w((lambda *s: _rng.normal(s) * 0.05)(D, F)),
            "w_up": _w((lambda *s: _rng.normal(s) * 0.05)(D, F)),
            "w_down": _w((lambda *s: _rng.normal(s) * 0.05)(F, D)),
        }
    _B_in = _B_setup()

    return {
        "A_x": _A_in["x"],
        "A_wq": _A_in["wq"],
        "A_wk": _A_in["wk"],
        "A_wv": _A_in["wv"],
        "A_wo": _A_in["wo"],
        "B_x": _B_in["x"],
        "B_w_gate": _B_in["w_gate"],
        "B_w_up": _B_in["w_up"],
        "B_w_down": _B_in["w_down"],
        "gate_w": _w((lambda *s: _rng.normal(s) * 0.05)(512) * 16.0),
    }

def reference(A_x, A_wq, A_wk, A_wv, A_wo, B_x, B_w_gate, B_w_up, B_w_down, gate_w):
    def _A_ref(x, wq, wk, wv, wo):
        B, S, D = x.shape
        H = 32
        Dh = D // H
        q = (lambda x, *d: x.transpose(*d))((x @ wq).reshape(B, S, H, Dh), 0, 2, 1, 3)
        k = x @ wk
        v = x @ wv
        scores = jnp.einsum("bhqd,bkd->bhqk", q, k) * (Dh ** -0.5)
        p = _softmax(scores, axis=-1)
        o = jnp.einsum("bhqk,bkd->bhqd", p, v)
        return (lambda x, *d: x.transpose(*d))(o, 0, 2, 1, 3).reshape(B, S, H * Dh) @ wo

    def _B_ref(x, w_gate, w_up, w_down):
        g = _silu(x @ w_gate)
        u = x @ w_up
        return (g * u) @ w_down

    x = A_x
    g = _sigmoid((x * gate_w).sum(-1, keepdims=True))
    a = _A_ref(x, A_wq, A_wk, A_wv, A_wo)
    b = _B_ref(x, B_w_gate, B_w_up, B_w_down)
    return g * a + (1 - g) * b
```

```python
import functools
import math
import jax
import jax.numpy as jnp
from jax import lax
import jax.experimental.pallas as pl
import jax.experimental.pallas.tpu as pltpu

BF = jnp.bfloat16
F32 = jnp.float32
NT_DIMS = (((1,), (1,)), ((), ()))
TN_NT_DIMS = (((0,), (1,)), ((), ()))


def _tree(parts, f):
    while len(parts) > 1:
        parts = [f(parts[i], parts[i + 1]) if i + 1 < len(parts) else parts[i] for i in range(0, len(parts), 2)]
    return parts[0]


def _tsum(p):
    return _tree([p[i * 8:(i + 1) * 8] for i in range(p.shape[0] // 8)], lambda a, b: a + b)


def _cmax(s):
    return s.reshape(s.shape[0] // 8, 8, s.shape[1]).max(axis=0)


def make_kernel_fn(TQ=512, CK=128, FC=256, G=4, gw1d=True, pvpos=0):
    def fn(A_x, A_wq, A_wk, A_wv, A_wo, B_x, B_w_gate, B_w_up, B_w_down, gate_w):
        B, S, D = A_x.shape
        H = 32
        Dh = D // H
        F = B_w_gate.shape[1]
        NB = S // TQ
        NC = S // CK
        NG = H // G
        NF = F // FC
        scale = (Dh ** -0.5) * math.log2(math.e)

        def kernel(x_ref, wq_ref, wkt_ref, wvt_ref, gw_ref, wo_hbm, wg_hbm, wu_hbm, wd_hbm, o_ref,
                   qt_ref, k_ref, vt_ref, sa_ref, sb_ref, m_ref, ot_ref, wo_ref, wg_ref, wu_ref, wd_ref, sems):
            j = pl.program_id(0)
            copies = [pltpu.make_async_copy(src, dst, sems.at[i]) for i, (src, dst) in enumerate(
                [(wg_hbm, wg_ref), (wu_hbm, wu_ref), (wd_hbm, wd_ref), (wo_hbm, wo_ref)])]

            @pl.when(j == 0)
            def _():
                for cp in copies:
                    cp.start()
                x = x_ref[...]
                k_ref[...] = lax.dot_general(x, wkt_ref[...], NT_DIMS, preferred_element_type=F32).astype(BF)
                vt_ref[...] = lax.dot_general(wvt_ref[...], x, NT_DIMS, preferred_element_type=F32).astype(BF)

            xb = x_ref[pl.ds(pl.multiple_of(j * TQ, TQ), TQ), :]

            def qk_chunk(c, q, s_out, mx):
                s = jnp.dot(k_ref[c * CK:(c + 1) * CK, :], q, preferred_element_type=F32)
                s_out[c * CK:(c + 1) * CK, :] = s
                sm = _cmax(s)
                return sm if mx is None else jnp.maximum(mx, sm)

            def make_ops(i_cur, s_cur, i_nxt, s_nxt):
                st = {}
                ms = [m_ref[g] for g in range(G)] if s_cur is not None else None

                def do_qk(n):
                    g, c = divmod(n, NC)
                    if c == 0:
                        st["q"] = qt_ref[i_nxt * G + g]
                        st["mx"] = None
                    st["mx"] = qk_chunk(c, st["q"], s_nxt.at[g], st["mx"])
                    if c == NC - 1:
                        m_ref[g] = st["mx"].max(axis=0, keepdims=True)

                def do_pv(n):
                    g, c = divmod(n, NC)
                    p = jnp.exp2(s_cur[g, c * CK:(c + 1) * CK, :] - ms[g])
                    ps = _tsum(p)
                    st["l"] = ps if c == 0 else st["l"] + ps
                    oc = jnp.dot(vt_ref[:, c * CK:(c + 1) * CK], p.astype(BF), preferred_element_type=F32)
                    st["o"] = oc if c == 0 else st["o"] + oc
                    if c == NC - 1:
                        linv = 1.0 / st["l"].sum(axis=0, keepdims=True)
                        h = i_cur * G + g
                        row = h * Dh if isinstance(h, int) else pl.multiple_of(h * Dh, Dh)
                        ot_ref[pl.ds(row, Dh), :] = st["o"] * linv
                return do_qk, do_pv

            qt = lax.dot_general(wq_ref[...], xb, TN_NT_DIMS, preferred_element_type=F32)
            qt_ref[...] = (qt * scale).astype(BF).reshape(H, Dh, TQ)

            @pl.when(j >= 0)
            def _():
                do_qk, _ = make_ops(None, None, 0, sa_ref)
                for n in range(G * NC):
                    do_qk(n)

            def group(i, s_cur, s_nxt):
                do_qk, do_pv = make_ops(i, s_cur, i + 1, s_nxt)
                for n in range(G * NC):
                    do_qk(n)
                    do_pv(n)

            def body(i, carry):
                @pl.when(i % 2 == 0)
                def _():
                    group(i, sa_ref, sb_ref)

                @pl.when(i % 2 == 1)
                def _():
                    group(i, sb_ref, sa_ref)
                return carry

            lax.fori_loop(0, NG - 1, body, 0)

            @pl.when(j == 0)
            def _():
                for cp in copies:
                    cp.wait()

            s_last = sa_ref if (NG - 1) % 2 == 0 else sb_ref
            _, do_pv = make_ops(NG - 1, s_last, None, None)
            NPV = G * NC
            per = -(-NPV // (3 * (NF - 1)))
            state = {"n": 0}

            def some_pv(k):
                for _ in range(k):
                    if state["n"] < NPV:
                        do_pv(state["n"])
                        state["n"] += 1

            bacc = None
            for f in range(NF):
                g = jnp.dot(xb, wg_ref[:, f * FC:(f + 1) * FC], preferred_element_type=F32)
                some_pv(per)
                u = jnp.dot(xb, wu_ref[:, f * FC:(f + 1) * FC], preferred_element_type=F32)
                some_pv(per)
                act = (g * jax.nn.sigmoid(g) * u).astype(BF)
                d = jnp.dot(act, wd_ref[f * FC:(f + 1) * FC, :], preferred_element_type=F32)
                some_pv(per)
                bacc = d if bacc is None else bacc + d
                if f == NF - 2:
                    some_pv(NPV)
                    on = ot_ref[...].T.astype(BF)
            a = jnp.dot(on, wo_ref[...], preferred_element_type=F32)
            gw = gw_ref[...].astype(F32).reshape(1, D)
            gl = jnp.sum(xb.astype(F32) * gw, axis=-1, keepdims=True)
            gate = jax.nn.sigmoid(gl)
            o_ref[...] = (gate * a + (1.0 - gate) * bacc).astype(o_ref.dtype)

        full = lambda shape: pl.BlockSpec(shape, lambda j: (0,) * len(shape), pipeline_mode=pl.Buffered(1))
        anyspec = pl.BlockSpec(memory_space=pl.ANY)
        gwa = gate_w if gw1d else gate_w.reshape(1, D)
        out = pl.pallas_call(
            kernel,
            grid=(NB,),
            in_specs=[
                full((S, D)), full((D, D)), full((Dh, D)), full((Dh, D)), full(gwa.shape),
                anyspec, anyspec, anyspec, anyspec,
            ],
            out_specs=pl.BlockSpec((TQ, D), lambda j: (j, 0)),
            out_shape=jax.ShapeDtypeStruct((S, D), A_x.dtype),
            scratch_shapes=[
                pltpu.VMEM((H, Dh, TQ), BF),
                pltpu.VMEM((S, Dh), BF),
                pltpu.VMEM((Dh, S), BF),
                pltpu.VMEM((G, S, TQ), F32),
                pltpu.VMEM((G, S, TQ), F32),
                pltpu.VMEM((G, 1, TQ), F32),
                pltpu.VMEM((D, TQ), F32),
                pltpu.VMEM((D, D), BF),
                pltpu.VMEM((D, F), BF),
                pltpu.VMEM((D, F), BF),
                pltpu.VMEM((F, D), BF),
                pltpu.SemaphoreType.DMA((4,)),
            ],
            compiler_params=pltpu.CompilerParams(
                dimension_semantics=("arbitrary",),
                vmem_limit_bytes=110 * 1024 * 1024,
            ),
        )(A_x.reshape(S, D), A_wq, A_wk.T, A_wv.T, gwa, A_wo, B_w_gate, B_w_up, B_w_down)
        return out.reshape(B, S, D)
    return jax.jit(fn)


_kernel_fn = make_kernel_fn()


@jax.jit
def pallas_gated_mix__grouped_kv_mqa__swiglu_ffn__prompt_kernel(
    A_x: jax.Array,
    A_wq: jax.Array,
    A_wk: jax.Array,
    A_wv: jax.Array,
    A_wo: jax.Array,
    B_x: jax.Array,
    B_w_gate: jax.Array,
    B_w_up: jax.Array,
    B_w_down: jax.Array,
    gate_w: jax.Array,
):
    return _kernel_fn(A_x, A_wq, A_wk, A_wv, A_wo, B_x, B_w_gate, B_w_up, B_w_down, gate_w)
```

```python
import math
import jax
import jax.numpy as jnp
from jax import lax
import jax.experimental.pallas as pl
import jax.experimental.pallas.tpu as pltpu

BF = jnp.bfloat16
F32 = jnp.float32
NT_DIMS = (((1,), (1,)), ((), ()))


def _tree(parts, f):
    while len(parts) > 1:
        parts = [f(parts[i], parts[i + 1]) if i + 1 < len(parts) else parts[i] for i in range(0, len(parts), 2)]
    return parts[0]


def _tsum(p):
    return _tree([p[i * 8:(i + 1) * 8] for i in range(p.shape[0] // 8)], lambda a, b: a + b)


def _cmax(s):
    return s.reshape(s.shape[0] // 8, 8, s.shape[1]).max(axis=0)


def make_kernel_fn(TQ=512, FC=256, G=4, NVK=160, C=3, A=64, A0=160, CB=128, MR=128, ktr=True, lag=1):
    CK = 128

    def fn(A_x, A_wq, A_wk, A_wv, A_wo, B_x, B_w_gate, B_w_up, B_w_down, gate_w):
        B, S, D = A_x.shape
        H = 32
        Dh = D // H
        F = B_w_gate.shape[1]
        NB = S // TQ
        NC = S // CK
        NG = H // G
        NF = F // FC
        NM = S - NVK
        J = TQ // 128
        R = NVK // 8
        NP = TQ // MR
        A1 = [A0] + [A] * (NC - 1)
        n1 = sum(A1)
        scale = (Dh ** -0.5) * math.log2(math.e)
        allo = [(r, jj) for jj in range(J) for r in range(R)]
        rounds = [allo[k:k + C] for k in range(0, len(allo), C)]

        def kernel(wkt_ref, wvt_ref, gw_ref, x_hbm, wq_hbm, wo_hbm, wg_hbm, wu_hbm, wd_hbm, o_ref,
                   x_ref, wq_ref, wo_ref, wg_ref, wu_ref, wd_ref, wp_ref,
                   qt_ref, qf_ref, k_ref, vt_ref, kb_ref, sa_ref, sb_ref, m_ref, ot_ref, sems):
            j = pl.program_id(0)
            wq_copy = pltpu.make_async_copy(wq_hbm, wq_ref, sems.at[0])
            x_copies = [pltpu.make_async_copy(x_hbm.at[pl.ds(b * TQ, TQ)], x_ref.at[pl.ds(b * TQ, TQ)], sems.at[1 + b])
                        for b in range(NB)]
            w_copies = [pltpu.make_async_copy(src, dst, sems.at[1 + NB + i]) for i, (src, dst) in enumerate(
                [(wg_hbm, wg_ref), (wu_hbm, wu_ref), (wd_hbm, wd_ref), (wo_hbm, wo_ref)])]

            @pl.when(j == 0)
            def _():
                wq_copy.start()
                for cp in x_copies:
                    cp.start()
                for cp in w_copies:
                    cp.start()
                wp_ref[D:D + Dh, :] = wkt_ref[...]
                wp_ref[D + Dh:D + 2 * Dh, :] = wvt_ref[...]
                wq_copy.wait()
                wp_ref[0:D, :] = wq_ref[...].T
                for b in range(NB):
                    x_copies[b].wait()
                    xb = x_ref[b * TQ:(b + 1) * TQ, :]
                    pr = lax.dot_general(wp_ref[...], xb, NT_DIMS, preferred_element_type=F32)
                    qb = (pr[0:D] * scale).astype(BF)
                    qt_ref[b * H:(b + 1) * H] = qb.reshape(H, Dh, TQ)
                    qf_ref[b * H:(b + 1) * H] = qb.astype(F32).reshape(H, Dh, TQ)
                    vt_ref[:, b * TQ:(b + 1) * TQ] = pr[D + Dh:D + 2 * Dh].astype(BF)
                    kb16 = pr[D:D + Dh].T.astype(BF)
                    k_ref[b * TQ:(b + 1) * TQ, :] = kb16
                    if b == NB - 1 and NVK:
                        kf = kb16[TQ - NVK:, :].astype(F32)
                        for d in range(Dh):
                            kb_ref[d] = jnp.broadcast_to(kf[:, d:d + 1], (NVK, 128))

            def make_ops(tag, i_cur, s_cur, i_nxt, s_nxt):
                never = lax.broadcasted_iota(jnp.int32, (8, 128), 1) > (tag + 4096)
                st = {}
                ms = [m_ref[g] for g in range(G)] if s_cur is not None else None
                mx = [None] * G
                qs = [None] * G
                pos = [0] * G
                vmx = [[[None] * J for u in range(C)] for g in range(G)]
                link = [None] * C

                def qk(g, n):
                    lo = pos[g]
                    hi = min(lo + n, NM)
                    pos[g] = hi
                    if hi <= lo:
                        return
                    if qs[g] is None:
                        qs[g] = qt_ref[j * H + i_nxt * G + g]
                    s = jnp.dot(k_ref[lo:hi, :], qs[g], preferred_element_type=F32)
                    s_nxt[g, lo:hi, :] = s
                    sm = _cmax(s)
                    mx[g] = sm if mx[g] is None else jnp.maximum(mx[g], sm)

                def vpu(g, lst):
                    t = j * H + i_nxt * G + g
                    for rnd in lst:
                        acc = [None] * len(rnd)
                        for d in range(Dh):
                            for u, (r, jj) in enumerate(rnd):
                                kk = kb_ref[d, r * 8:r * 8 + 8, :]
                                qq = jnp.broadcast_to(qf_ref[t, d:d + 1, jj * 128:(jj + 1) * 128], (8, 128))
                                tt = kk * qq
                                if acc[u] is None:
                                    acc[u] = tt if link[u] is None else jnp.where(never, link[u], tt)
                                else:
                                    acc[u] = acc[u] + tt
                        for u, (r, jj) in enumerate(rnd):
                            s_nxt[g, NM + r * 8:NM + r * 8 + 8, jj * 128:(jj + 1) * 128] = acc[u]
                            v = vmx[g][u][jj]
                            v = acc[u] if v is None else jnp.maximum(v, acc[u])
                            vmx[g][u][jj] = v
                            link[u] = v

                def fin(g):
                    m = mx[g]
                    if NVK:
                        cols = [_tree([vmx[g][u][jj] for u in range(C) if vmx[g][u][jj] is not None], jnp.maximum)
                                for jj in range(J)]
                        m = jnp.maximum(m, jnp.concatenate(cols, axis=1))
                    m_ref[g] = m.max(axis=0, keepdims=True)

                def qk_rest(g):
                    rem = NM - pos[g]
                    n2 = -(-rem // CB)
                    for c in range(n2):
                        qk(g, CB)
                        vpu(g, rounds[(len(rounds) * c) // n2:(len(rounds) * (c + 1)) // n2])
                    fin(g)

                def pv(g, c):
                    p = jnp.exp2(s_cur[g, c * CK:(c + 1) * CK, :] - ms[g])
                    ps = _tsum(p)
                    st["l"] = ps if c == 0 else st["l"] + ps
                    oc = jnp.dot(vt_ref[:, c * CK:(c + 1) * CK], p.astype(BF), preferred_element_type=F32)
                    st["o"] = oc if c == 0 else st["o"] + oc
                    if c == NC - 1:
                        linv = 1.0 / st["l"].sum(axis=0, keepdims=True)
                        h = i_cur * G + g
                        row = h * Dh if isinstance(h, int) else pl.multiple_of(h * Dh, Dh)
                        ot_ref[pl.ds(row, Dh), :] = st["o"] * linv
                return qk, qk_rest, pv

            @pl.when(j >= 0)
            def _():
                _, qk_rest, _ = make_ops(j, None, None, 0, sa_ref)
                for g in range(G):
                    qk_rest(g)

            def group(i, s_cur, s_nxt):
                qk, qk_rest, pv = make_ops(i, i, s_cur, i + 1, s_nxt)
                for g in range(G):
                    for c in range(NC):
                        qk(g, A1[c])
                        pv(g, c)
                    qk_rest(g)

            def body(i, carry):
                @pl.when(i % 2 == 0)
                def _():
                    group(i, sa_ref, sb_ref)

                @pl.when(i % 2 == 1)
                def _():
                    group(i, sb_ref, sa_ref)
                return carry

            lax.fori_loop(0, NG - 1, body, 0)

            @pl.when(j == 0)
            def _():
                for cp in w_copies:
                    cp.wait()

            s_last = sa_ref if (NG - 1) % 2 == 0 else sb_ref
            _, _, pv = make_ops(j, NG - 1, s_last, None, None)
            NPV = G * NC
            state = {"n": 0}

            def some_pv():
                if state["n"] < NPV:
                    pv(*divmod(state["n"], NC))
                    state["n"] += 1

            row0 = pl.multiple_of(j * TQ, TQ)
            bacc = [None] * NP
            pend = []

            def down():
                pp, ff, aa = pend.pop(0)
                d = jnp.dot(aa, wd_ref[ff * FC:(ff + 1) * FC, :], preferred_element_type=F32)
                some_pv()
                bacc[pp] = d if bacc[pp] is None else bacc[pp] + d

            xs = []
            for p in range(NP):
                xp = x_ref[pl.ds(row0 + p * MR, MR), :]
                xs.append(xp)
                for f in range(NF):
                    g = jnp.dot(xp, wg_ref[:, f * FC:(f + 1) * FC], preferred_element_type=F32)
                    some_pv()
                    u = jnp.dot(xp, wu_ref[:, f * FC:(f + 1) * FC], preferred_element_type=F32)
                    some_pv()
                    hh = 0.5 * g
                    act = ((hh + hh * jnp.tanh(hh)) * u).astype(BF)
                    pend.append((p, f, act))
                    if len(pend) > lag:
                        down()
            while pend:
                down()
            while state["n"] < NPV:
                some_pv()
            gw = gw_ref[...].astype(F32).reshape(1, D)
            for p in range(NP):
                on = ot_ref[:, p * MR:(p + 1) * MR].T.astype(BF)
                a = jnp.dot(on, wo_ref[...], preferred_element_type=F32)
                gl = jnp.sum(xs[p].astype(F32) * gw, axis=-1, keepdims=True)
                gate = 0.5 + 0.5 * jnp.tanh(0.5 * gl)
                o_ref[p * MR:(p + 1) * MR, :] = (bacc[p] + gate * (a - bacc[p])).astype(o_ref.dtype)

        full = lambda shape: pl.BlockSpec(shape, lambda j: (0,) * len(shape), pipeline_mode=pl.Buffered(1))
        anyspec = pl.BlockSpec(memory_space=pl.ANY)
        out = pl.pallas_call(
            kernel,
            grid=(NB,),
            in_specs=[full((Dh, D)), full((Dh, D)), full((D,))] + [anyspec] * 6,
            out_specs=pl.BlockSpec((TQ, D), lambda j: (j, 0)),
            out_shape=jax.ShapeDtypeStruct((S, D), A_x.dtype),
            scratch_shapes=[
                pltpu.VMEM((S, D), BF),
                pltpu.VMEM((D, D), BF),
                pltpu.VMEM((D, D), BF),
                pltpu.VMEM((D, F), BF),
                pltpu.VMEM((D, F), BF),
                pltpu.VMEM((F, D), BF),
                pltpu.VMEM((D + 2 * Dh, D), BF),
                pltpu.VMEM((NB * H, Dh, TQ), BF),
                pltpu.VMEM((NB * H, Dh, TQ), F32),
                pltpu.VMEM((S, Dh), BF),
                pltpu.VMEM((Dh, S), BF),
                pltpu.VMEM((Dh, max(NVK, 8), 128), F32),
                pltpu.VMEM((G, S, TQ), F32),
                pltpu.VMEM((G, S, TQ), F32),
                pltpu.VMEM((G, 1, TQ), F32),
                pltpu.VMEM((D, TQ), F32),
                pltpu.SemaphoreType.DMA((1 + NB + 4,)),
            ],
            compiler_params=pltpu.CompilerParams(
                dimension_semantics=("arbitrary",),
                vmem_limit_bytes=110 * 1024 * 1024,
            ),
        )(A_wk.T, A_wv.T, gate_w, A_x.reshape(S, D), A_wq, A_wo, B_w_gate, B_w_up, B_w_down)
        return out.reshape(B, S, D)
    return jax.jit(fn)


_kernel_fn = make_kernel_fn()


@jax.jit
def pallas_gated_mix__grouped_kv_mqa__swiglu_ffn__prompt_kernel(
    A_x: jax.Array,
    A_wq: jax.Array,
    A_wk: jax.Array,
    A_wv: jax.Array,
    A_wo: jax.Array,
    B_x: jax.Array,
    B_w_gate: jax.Array,
    B_w_up: jax.Array,
    B_w_down: jax.Array,
    gate_w: jax.Array,
):
    return _kernel_fn(A_x, A_wq, A_wk, A_wv, A_wo, B_x, B_w_gate, B_w_up, B_w_down, gate_w)
```

```python
import math

import jax
import jax.numpy as jnp
from jax import lax
import jax.experimental.pallas as pl
import jax.experimental.pallas.tpu as pltpu

BF = jnp.bfloat16
F32 = jnp.float32
NT_DIMS = (((1,), (1,)), ((), ()))

H = 32
TQ = 512
G = 4
NV_LOOP = 160
NV_FIRST = 304
CHAINS = 3
PV_LEAD = (64, 64)
QK_LEAD = (144, 48)
QK_STEP = 64
QK_REST = 96
MR = 128
FC = 128


def _tree(parts, f):
    while len(parts) > 1:
        parts = [f(parts[i], parts[i + 1]) if i + 1 < len(parts) else parts[i]
                 for i in range(0, len(parts), 2)]
    return parts[0]


def _group_sum(p):
    return _tree([p[i * 8:(i + 1) * 8] for i in range(p.shape[0] // 8)], lambda a, b: a + b)


def _group_max(s):
    return s.reshape(s.shape[0] // 8, 8, s.shape[1]).max(axis=0)


@jax.jit
def pallas_gated_mix__grouped_kv_mqa__swiglu_ffn__prompt_kernel(
    A_x: jax.Array,
    A_wq: jax.Array,
    A_wk: jax.Array,
    A_wv: jax.Array,
    A_wo: jax.Array,
    B_x: jax.Array,
    B_w_gate: jax.Array,
    B_w_up: jax.Array,
    B_w_down: jax.Array,
    gate_w: jax.Array,
):
    del B_x
    B, S, D = A_x.shape
    assert B == 1
    Dh = D // H
    F = B_w_gate.shape[1]
    NB = S // TQ
    NG = H // G
    NF = F // FC
    J = TQ // 128
    NP = TQ // MR
    NKB = max(NV_LOOP, NV_FIRST)
    assert NKB <= TQ
    pvb = [0]
    for w in PV_LEAD:
        pvb.append(pvb[-1] + w)
    while pvb[-1] < S:
        pvb.append(min(S, pvb[-1] + 128))
    NC = len(pvb) - 1
    qk_sizes = list(QK_LEAD) + [QK_STEP] * (NC - len(QK_LEAD))
    scale = (Dh ** -0.5) * math.log2(math.e)
    order = [NB - 1] + list(range(NB - 1))

    def kernel(wkt_ref, wvt_ref, gw_ref, x_hbm, wq_hbm, wo_hbm, wg_hbm, wu_hbm, wd_hbm, o_ref,
               x_ref, wq_ref, wo_ref, wg_ref, wu_ref, wd_ref, wp_ref,
               qt_ref, qf_ref, k_ref, vt_ref, kb_ref, sa_ref, sb_ref, m_ref, ot_ref, sems):
        j = pl.program_id(0)
        wq_copy = pltpu.make_async_copy(wq_hbm, wq_ref, sems.at[0])
        x_copies = [
            pltpu.make_async_copy(x_hbm.at[pl.ds(b * TQ, TQ)], x_ref.at[pl.ds(b * TQ, TQ)], sems.at[1 + b])
            for b in range(NB)]
        w_copies = [
            pltpu.make_async_copy(src, dst, sems.at[1 + NB + i])
            for i, (src, dst) in enumerate(
                [(wg_hbm, wg_ref), (wu_hbm, wu_ref), (wd_hbm, wd_ref), (wo_hbm, wo_ref)])]

        @pl.when(j == 0)
        def _():
            wq_copy.start()
            x_copies[order[0]].start()
            wp_ref[D:D + Dh, :] = wkt_ref[...]
            wp_ref[D + Dh:D + 2 * Dh, :] = wvt_ref[...]
            wq_copy.wait()
            for b in order[1:]:
                x_copies[b].start()
            wp_ref[0:D, :] = wq_ref[...].T
            kf = None
            for n, b in enumerate(order):
                if n == 0:
                    x_copies[b].wait()
                    for cp in w_copies:
                        cp.start()
                if n == 1:
                    for bb in order[1:]:
                        x_copies[bb].wait()
                    for d in range(Dh):
                        kb_ref[d] = jnp.broadcast_to(kf[:, d:d + 1], (NKB, 128))
                xb = x_ref[b * TQ:(b + 1) * TQ, :]
                pr = lax.dot_general(wp_ref[...], xb, NT_DIMS, preferred_element_type=F32)
                qb = (pr[0:D] * scale).astype(BF)
                qt_ref[b * H:(b + 1) * H] = qb.reshape(H, Dh, TQ)
                qf_ref[b * H:(b + 1) * H] = qb.astype(F32).reshape(H, Dh, TQ)
                vt_ref[:, b * TQ:(b + 1) * TQ] = pr[D + Dh:D + 2 * Dh].astype(BF)
                kb16 = pr[D:D + Dh].T.astype(BF)
                k_ref[b * TQ:(b + 1) * TQ, :] = kb16
                if n == 0:
                    kf = kb16[TQ - NKB:, :].astype(F32)

        def make_ops(tag, i_cur, s_cur, i_nxt, s_nxt, nv):
            nm = S - nv
            r0 = (NKB - nv) // 8
            outs = [(r, jj) for jj in range(J) for r in range(nv // 8)]
            rounds = [outs[k:k + CHAINS] for k in range(0, len(outs), CHAINS)]
            never = lax.broadcasted_iota(jnp.int32, (8, 128), 1) > (tag + 4096)
            st = {}
            ms = [m_ref[g] for g in range(G)] if s_cur is not None else None
            mx = [None] * G
            qs = [None] * G
            pos = [0] * G

            def qk(g, n):
                lo = pos[g]
                hi = min(lo + n, nm)
                pos[g] = hi
                if hi <= lo:
                    return
                if qs[g] is None:
                    qs[g] = qt_ref[j * H + i_nxt * G + g]
                s = jnp.dot(k_ref[lo:hi, :], qs[g], preferred_element_type=F32)
                s_nxt[g, lo:hi, :] = s
                sm = _group_max(s)
                mx[g] = sm if mx[g] is None else jnp.maximum(mx[g], sm)

            def qk_rest(g):
                t = j * H + i_nxt * G + g
                vmx = [[None] * J for _ in range(CHAINS)]
                link = [None] * CHAINS
                n2 = -(-(nm - pos[g]) // QK_REST)
                for c in range(n2):
                    qk(g, QK_REST)
                    for rnd in rounds[(len(rounds) * c) // n2:(len(rounds) * (c + 1)) // n2]:
                        acc = [None] * len(rnd)
                        for d in range(Dh):
                            for u, (r, jj) in enumerate(rnd):
                                kk = kb_ref[d, (r0 + r) * 8:(r0 + r) * 8 + 8, :]
                                qq = jnp.broadcast_to(
                                    qf_ref[t, d:d + 1, jj * 128:(jj + 1) * 128], (8, 128))
                                tt = kk * qq
                                if acc[u] is None:
                                    acc[u] = tt if link[u] is None else jnp.where(never, link[u], tt)
                                else:
                                    acc[u] = acc[u] + tt
                        for u, (r, jj) in enumerate(rnd):
                            s_nxt[g, nm + r * 8:nm + r * 8 + 8, jj * 128:(jj + 1) * 128] = acc[u]
                            v = vmx[u][jj]
                            v = acc[u] if v is None else jnp.maximum(v, acc[u])
                            vmx[u][jj] = v
                            link[u] = v
                cols = [_tree([vmx[u][jj] for u in range(CHAINS) if vmx[u][jj] is not None], jnp.maximum)
                        for jj in range(J)]
                m = jnp.maximum(mx[g], jnp.concatenate(cols, axis=1))
                m_ref[g] = m.max(axis=0, keepdims=True)

            def pv(g, c):
                lo, hi = pvb[c], pvb[c + 1]
                p = jnp.exp2(s_cur[g, lo:hi, :] - ms[g])
                ps = _group_sum(p)
                st["l"] = ps if c == 0 else st["l"] + ps
                oc = jnp.dot(vt_ref[:, lo:hi], p.astype(BF), preferred_element_type=F32)
                st["o"] = oc if c == 0 else st["o"] + oc
                if c == NC - 1:
                    linv = 1.0 / st["l"].sum(axis=0, keepdims=True)
                    h = i_cur * G + g
                    row = h * Dh if isinstance(h, int) else pl.multiple_of(h * Dh, Dh)
                    ot_ref[pl.ds(row, Dh), :] = st["o"] * linv

            return qk, qk_rest, pv

        @pl.when(j >= 0)
        def _():
            _, qk_rest, _ = make_ops(j, None, None, 0, sa_ref, NV_FIRST)
            for g in range(G):
                qk_rest(g)

        def group(i, s_cur, s_nxt):
            qk, qk_rest, pv = make_ops(i, i, s_cur, i + 1, s_nxt, NV_LOOP)
            for g in range(G):
                for c in range(NC):
                    qk(g, qk_sizes[c])
                    pv(g, c)
                qk_rest(g)

        def body(i, carry):
            @pl.when(i % 2 == 0)
            def _():
                group(i, sa_ref, sb_ref)

            @pl.when(i % 2 == 1)
            def _():
                group(i, sb_ref, sa_ref)
            return carry

        lax.fori_loop(0, NG - 1, body, 0)

        @pl.when(j == 0)
        def _():
            for cp in w_copies:
                cp.wait()

        s_last = sa_ref if (NG - 1) % 2 == 0 else sb_ref
        _, _, pv = make_ops(j, NG - 1, s_last, None, None, 0)
        n_pv = G * NC
        done = [0]

        def one_pv():
            if done[0] < n_pv:
                pv(*divmod(done[0], NC))
                done[0] += 1

        row0 = pl.multiple_of(j * TQ, TQ)
        bacc = [None] * NP
        pend = []

        def down():
            pp, ff, aa = pend.pop(0)
            d = jnp.dot(aa, wd_ref[ff * FC:(ff + 1) * FC, :], preferred_element_type=F32)
            one_pv()
            bacc[pp] = d if bacc[pp] is None else bacc[pp] + d

        xs = []
        for p in range(NP):
            xp = x_ref[pl.ds(row0 + p * MR, MR), :]
            xs.append(xp)
            for f in range(NF):
                g = jnp.dot(xp, wg_ref[:, f * FC:(f + 1) * FC], preferred_element_type=F32)
                one_pv()
                u = jnp.dot(xp, wu_ref[:, f * FC:(f + 1) * FC], preferred_element_type=F32)
                one_pv()
                act = (g * u * pl.reciprocal(1.0 + jnp.exp(-g), approx=True)).astype(BF)
                pend.append((p, f, act))
                if len(pend) > 1:
                    down()
        while pend:
            down()
        while done[0] < n_pv:
            one_pv()
        gw = gw_ref[...].astype(F32).reshape(1, D)
        for p in range(NP):
            on = ot_ref[:, p * MR:(p + 1) * MR].T.astype(BF)
            a = jnp.dot(on, wo_ref[...], preferred_element_type=F32)
            gl = jnp.sum(xs[p].astype(F32) * gw, axis=-1, keepdims=True)
            gate = jax.nn.sigmoid(gl)
            o_ref[p * MR:(p + 1) * MR, :] = (gate * a + (1.0 - gate) * bacc[p]).astype(o_ref.dtype)

    def full(shape):
        return pl.BlockSpec(shape, lambda j: (0,) * len(shape), pipeline_mode=pl.Buffered(1))

    hbm = pl.BlockSpec(memory_space=pl.ANY)
    out = pl.pallas_call(
        kernel,
        grid=(NB,),
        in_specs=[full((Dh, D)), full((Dh, D)), full((D,))] + [hbm] * 6,
        out_specs=pl.BlockSpec((TQ, D), lambda j: (j, 0)),
        out_shape=jax.ShapeDtypeStruct((S, D), A_x.dtype),
        scratch_shapes=[
            pltpu.VMEM((S, D), BF),
            pltpu.VMEM((D, D), BF),
            pltpu.VMEM((D, D), BF),
            pltpu.VMEM((D, F), BF),
            pltpu.VMEM((D, F), BF),
            pltpu.VMEM((F, D), BF),
            pltpu.VMEM((D + 2 * Dh, D), BF),
            pltpu.VMEM((NB * H, Dh, TQ), BF),
            pltpu.VMEM((NB * H, Dh, TQ), F32),
            pltpu.VMEM((S, Dh), BF),
            pltpu.VMEM((Dh, S), BF),
            pltpu.VMEM((Dh, NKB, 128), F32),
            pltpu.VMEM((G, S, TQ), F32),
            pltpu.VMEM((G, S, TQ), F32),
            pltpu.VMEM((G, 1, TQ), F32),
            pltpu.VMEM((D, TQ), F32),
            pltpu.SemaphoreType.DMA((1 + NB + 4,)),
        ],
        compiler_params=pltpu.CompilerParams(
            dimension_semantics=("arbitrary",),
            vmem_limit_bytes=100 * 1024 * 1024,
        ),
    )(A_wk.T, A_wv.T, gate_w, A_x.reshape(S, D), A_wq, A_wo, B_w_gate, B_w_up, B_w_down)
    return out.reshape(B, S, D)
```

```python
import math

import jax
import jax.numpy as jnp
from jax import lax
import jax.experimental.pallas as pl
import jax.experimental.pallas.tpu as pltpu

BF = jnp.bfloat16
F32 = jnp.float32
NT_DIMS = (((1,), (1,)), ((), ()))

H = 32
TQ = 512
G = 4
NV_LOOP = 160
NV_FIRST = 256
NV_AHEAD = 352
CHAINS = 3
CHAINS_AHEAD = 2
PV_LEAD = (64, 64)
QK_LEAD = (144, 48)
QK_STEP = 64
QK_REST = 96
MR = 128
FC = 128
AHEAD_START = 69
AHEAD_RATE = 3.4


def _tree(parts, f):
    while len(parts) > 1:
        parts = [f(parts[i], parts[i + 1]) if i + 1 < len(parts) else parts[i]
                 for i in range(0, len(parts), 2)]
    return parts[0]


def _group_sum(p):
    return _tree([p[i * 8:(i + 1) * 8] for i in range(p.shape[0] // 8)], lambda a, b: a + b)


def _group_max(s):
    return s.reshape(s.shape[0] // 8, 8, s.shape[1]).max(axis=0)


@jax.jit
def pallas_gated_mix__grouped_kv_mqa__swiglu_ffn__prompt_kernel(
    A_x: jax.Array,
    A_wq: jax.Array,
    A_wk: jax.Array,
    A_wv: jax.Array,
    A_wo: jax.Array,
    B_x: jax.Array,
    B_w_gate: jax.Array,
    B_w_up: jax.Array,
    B_w_down: jax.Array,
    gate_w: jax.Array,
):
    del B_x
    B, S, D = A_x.shape
    assert B == 1
    Dh = D // H
    F = B_w_gate.shape[1]
    NB = S // TQ
    NG = H // G
    NF = F // FC
    J = TQ // 128
    NP = TQ // MR
    NS = NV_AHEAD
    NKB = NV_FIRST + NS
    assert NV_LOOP <= NKB and TQ < NKB <= 2 * TQ and NS <= TQ and NG % 2 == 0
    pvb = [0]
    for w in PV_LEAD:
        pvb.append(pvb[-1] + w)
    while pvb[-1] < S:
        pvb.append(min(S, pvb[-1] + 128))
    NC = len(pvb) - 1
    qk_sizes = list(QK_LEAD) + [QK_STEP] * (NC - len(QK_LEAD))
    scale = (Dh ** -0.5) * math.log2(math.e)
    order = [NB - 1, NB - 2] + list(range(NB - 2))

    def kernel(wkt_ref, wvt_ref, gw_ref, x_hbm, wq_hbm, wo_hbm, wg_hbm, wu_hbm, wd_hbm, o_ref,
               x_ref, wq_ref, wo_ref, wg_ref, wu_ref, wd_ref, wp_ref,
               qt_ref, qf_ref, k_ref, vt_ref, kb_ref, sa_ref, sb_ref, m_ref, ot_ref, ma_ref, sems):
        j = pl.program_id(0)
        wq_copy = pltpu.make_async_copy(wq_hbm, wq_ref, sems.at[0])
        x_copies = [
            pltpu.make_async_copy(x_hbm.at[pl.ds(b * TQ, TQ)], x_ref.at[pl.ds(b * TQ, TQ)], sems.at[1 + b])
            for b in range(NB)]
        w_copies = [
            pltpu.make_async_copy(src, dst, sems.at[1 + NB + i])
            for i, (src, dst) in enumerate(
                [(wg_hbm, wg_ref), (wu_hbm, wu_ref), (wd_hbm, wd_ref), (wo_hbm, wo_ref)])]

        @pl.when(j == 0)
        def _():
            wq_copy.start()
            x_copies[order[0]].start()
            wp_ref[D:D + Dh, :] = wkt_ref[...]
            wp_ref[D + Dh:D + 2 * Dh, :] = wvt_ref[...]
            wq_copy.wait()
            for b in order[1:]:
                x_copies[b].start()
            wp_ref[0:D, :] = wq_ref[...].T
            kf = ks = q0 = None
            for n, b in enumerate(order):
                if n == 0:
                    x_copies[b].wait()
                    for cp in w_copies:
                        cp.start()
                if n == 1:
                    for bb in order[1:]:
                        x_copies[bb].wait()
                    for d in range(Dh):
                        kb_ref[d, NKB - TQ:, :] = jnp.broadcast_to(kf[:, d:d + 1], (TQ, 128))
                if n == 2:
                    for d in range(Dh):
                        kb_ref[d, :NKB - TQ, :] = jnp.broadcast_to(kf[:, d:d + 1], (NKB - TQ, 128))
                xb = x_ref[b * TQ:(b + 1) * TQ, :]
                pr = lax.dot_general(wp_ref[...], xb, NT_DIMS, preferred_element_type=F32)
                qb = (pr[0:D] * scale).astype(BF)
                qt_ref[b * H:(b + 1) * H] = qb.reshape(H, Dh, TQ)
                qf_ref[b * H:(b + 1) * H] = qb.astype(F32).reshape(H, Dh, TQ)
                vt_ref[:, b * TQ:(b + 1) * TQ] = pr[D + Dh:D + 2 * Dh].astype(BF)
                kb16 = pr[D:D + Dh].T.astype(BF)
                k_ref[b * TQ:(b + 1) * TQ, :] = kb16
                if n == 0:
                    kf = kb16.astype(F32)
                    ks = kb16[TQ - NS:, :]
                if n == 1:
                    kf = kb16[2 * TQ - NKB:, :].astype(F32)
                if b == 0:
                    q0 = qb
            for g in range(G):
                mxs = None
                for c in range(0, NS, 128):
                    hi = min(NS, c + 128)
                    s = jnp.dot(ks[c:hi], q0[g * Dh:(g + 1) * Dh], preferred_element_type=F32)
                    sa_ref[g, S - NS + c:S - NS + hi, :] = s
                    mxs = _group_max(s) if mxs is None else jnp.maximum(mxs, _group_max(s))
                ma_ref[g] = mxs

        def never_mask(tag):
            return lax.broadcasted_iota(jnp.int32, (8, 128), 1) > (tag + 4096)

        def vpu_round(rnd, link, never):
            acc = [None] * len(rnd)
            for d in range(Dh):
                for u, (t, kr, jj) in enumerate(rnd):
                    kk = kb_ref[d, kr * 8:kr * 8 + 8, :]
                    qq = jnp.broadcast_to(qf_ref[t, d:d + 1, jj * 128:(jj + 1) * 128], (8, 128))
                    tt = kk * qq
                    if acc[u] is None:
                        acc[u] = tt if link[u] is None else jnp.where(never, link[u], tt)
                    else:
                        acc[u] = acc[u] + tt
            return acc

        def make_ops(tag, i_cur, s_cur, i_nxt, s_nxt, nv, ns=0):
            nm = S - nv - ns
            r0 = (NKB - nv - ns) // 8
            outs = [(r, jj) for jj in range(J) for r in range(nv // 8)]
            rounds = [outs[k:k + CHAINS] for k in range(0, len(outs), CHAINS)]
            never = never_mask(tag)
            st = {}
            ms = [m_ref[g] for g in range(G)] if s_cur is not None else None
            mx = [None] * G
            qs = [None] * G
            pos = [0] * G

            def qk(g, n):
                lo = pos[g]
                hi = min(lo + n, nm)
                pos[g] = hi
                if hi <= lo:
                    return
                if qs[g] is None:
                    qs[g] = qt_ref[j * H + i_nxt * G + g]
                s = jnp.dot(k_ref[lo:hi, :], qs[g], preferred_element_type=F32)
                s_nxt[g, lo:hi, :] = s
                sm = _group_max(s)
                mx[g] = sm if mx[g] is None else jnp.maximum(mx[g], sm)

            def qk_rest(g):
                t = j * H + i_nxt * G + g
                vmx = [[None] * J for _ in range(CHAINS)]
                link = [None] * CHAINS
                n2 = -(-(nm - pos[g]) // QK_REST)
                for c in range(n2):
                    qk(g, QK_REST)
                    for rnd in rounds[(len(rounds) * c) // n2:(len(rounds) * (c + 1)) // n2]:
                        acc = vpu_round([(t, r0 + r, jj) for r, jj in rnd], link, never)
                        for u, (r, jj) in enumerate(rnd):
                            s_nxt[g, nm + r * 8:nm + r * 8 + 8, jj * 128:(jj + 1) * 128] = acc[u]
                            v = vmx[u][jj]
                            v = acc[u] if v is None else jnp.maximum(v, acc[u])
                            vmx[u][jj] = v
                            link[u] = v
                cols = [_tree([vmx[u][jj] for u in range(CHAINS) if vmx[u][jj] is not None], jnp.maximum)
                        for jj in range(J)]
                m = jnp.maximum(mx[g], jnp.concatenate(cols, axis=1))
                if ns:
                    m = jnp.maximum(m, ma_ref[g])
                m_ref[g] = m.max(axis=0, keepdims=True)

            def pv(g, c):
                lo, hi = pvb[c], pvb[c + 1]
                p = jnp.exp2(s_cur[g, lo:hi, :] - ms[g])
                ps = _group_sum(p)
                st["l"] = ps if c == 0 else st["l"] + ps
                oc = jnp.dot(vt_ref[:, lo:hi], p.astype(BF), preferred_element_type=F32)
                st["o"] = oc if c == 0 else st["o"] + oc
                if c == NC - 1:
                    linv = 1.0 / st["l"].sum(axis=0, keepdims=True)
                    h = i_cur * G + g
                    row = h * Dh if isinstance(h, int) else pl.multiple_of(h * Dh, Dh)
                    ot_ref[pl.ds(row, Dh), :] = st["o"] * linv

            return qk, qk_rest, pv

        @pl.when(j >= 0)
        def _():
            _, qk_rest, _ = make_ops(j, None, None, 0, sa_ref, NV_FIRST, NS)
            for g in range(G):
                qk_rest(g)

        def group(i, s_cur, s_nxt):
            qk, qk_rest, pv = make_ops(i, i, s_cur, i + 1, s_nxt, NV_LOOP)
            for g in range(G):
                for c in range(NC):
                    qk(g, qk_sizes[c])
                    pv(g, c)
                qk_rest(g)

        def body(i, carry):
            @pl.when(i % 2 == 0)
            def _():
                group(i, sa_ref, sb_ref)

            @pl.when(i % 2 == 1)
            def _():
                group(i, sb_ref, sa_ref)
            return carry

        lax.fori_loop(0, NG - 1, body, 0)

        @pl.when(j == 0)
        def _():
            for cp in w_copies:
                cp.wait()

        _, _, pv = make_ops(j, NG - 1, sb_ref, None, None, 0)
        n_pv = G * NC
        jn = jnp.minimum(j + 1, NB - 1)
        never = never_mask(j)
        ahead = [(g, r, jj) for g in range(G) for jj in range(J) for r in range(NS // 8)]
        ahead_rounds = [ahead[k:k + CHAINS_AHEAD] for k in range(0, len(ahead), CHAINS_AHEAD)]
        link = [None] * CHAINS_AHEAD
        amx = {}
        state = {"pv": 0, "piece": 0, "round": 0}
        row0 = pl.multiple_of(j * TQ, TQ)
        xs = [x_ref[pl.ds(row0 + p * MR, MR), :] for p in range(NP)]
        gw = gw_ref[...].astype(F32).reshape(1, D)
        pre = {}

        def look_ahead(upto):
            while state["round"] < min(upto, len(ahead_rounds)):
                if state["round"] == 0:
                    assert state["pv"] == n_pv
                    pre["on"] = [ot_ref[:, p * MR:(p + 1) * MR].T.astype(BF) for p in range(NP)]
                    pre["gate"] = [
                        jax.nn.sigmoid(jnp.sum(xs[p].astype(F32) * gw, axis=-1, keepdims=True))
                        for p in range(NP)]
                    toks = [pltpu.bitcast(o[MR - 16:, D - 128:], F32) for o in pre["on"]]
                    toks += [jnp.broadcast_to(gt[MR - 8:], (8, 128)) for gt in pre["gate"]]
                    link[:] = [_tree(toks, jnp.maximum)] * CHAINS_AHEAD
                rnd = ahead_rounds[state["round"]]
                state["round"] += 1
                acc = vpu_round([(jn * H + g, (NKB - NS) // 8 + r, jj) for g, r, jj in rnd], link, never)
                for u, (g, r, jj) in enumerate(rnd):
                    sa_ref[g, S - NS + r * 8:S - NS + r * 8 + 8, jj * 128:(jj + 1) * 128] = acc[u]
                    v = amx.get((u, g, jj))
                    v = acc[u] if v is None else jnp.maximum(v, acc[u])
                    amx[(u, g, jj)] = v
                    link[u] = v
                    if r == NS // 8 - 1:
                        ma_ref[g, :, jj * 128:(jj + 1) * 128] = _tree(
                            [amx[(uu, g, jj)] for uu in range(CHAINS_AHEAD) if (uu, g, jj) in amx],
                            jnp.maximum)

        def after_piece():
            if state["pv"] < n_pv:
                pv(*divmod(state["pv"], NC))
                state["pv"] += 1
            state["piece"] += 1
            if state["piece"] > AHEAD_START:
                look_ahead(int(AHEAD_RATE * (state["piece"] - AHEAD_START)))

        bacc = [None] * NP
        pend = []

        def down():
            pp, ff, aa = pend.pop(0)
            d = jnp.dot(aa, wd_ref[ff * FC:(ff + 1) * FC, :], preferred_element_type=F32)
            after_piece()
            bacc[pp] = d if bacc[pp] is None else bacc[pp] + d

        for p in range(NP):
            for f in range(NF):
                g = jnp.dot(xs[p], wg_ref[:, f * FC:(f + 1) * FC], preferred_element_type=F32)
                after_piece()
                u = jnp.dot(xs[p], wu_ref[:, f * FC:(f + 1) * FC], preferred_element_type=F32)
                after_piece()
                act = (g * u * pl.reciprocal(1.0 + jnp.exp(-g), approx=True)).astype(BF)
                pend.append((p, f, act))
                if len(pend) > 1:
                    down()
        while pend:
            down()
        for p in range(NP):
            a = jnp.dot(pre["on"][p], wo_ref[...], preferred_element_type=F32)
            state["piece"] += 4
            look_ahead(int(AHEAD_RATE * (state["piece"] - AHEAD_START)) if p < NP - 1
                       else len(ahead_rounds))
            gate = pre["gate"][p]
            o_ref[p * MR:(p + 1) * MR, :] = (gate * a + (1.0 - gate) * bacc[p]).astype(o_ref.dtype)

    def full(shape):
        return pl.BlockSpec(shape, lambda j: (0,) * len(shape), pipeline_mode=pl.Buffered(1))

    hbm = pl.BlockSpec(memory_space=pl.ANY)
    out = pl.pallas_call(
        kernel,
        grid=(NB,),
        in_specs=[full((Dh, D)), full((Dh, D)), full((D,))] + [hbm] * 6,
        out_specs=pl.BlockSpec((TQ, D), lambda j: (j, 0)),
        out_shape=jax.ShapeDtypeStruct((S, D), A_x.dtype),
        scratch_shapes=[
            pltpu.VMEM((S, D), BF),
            pltpu.VMEM((D, D), BF),
            pltpu.VMEM((D, D), BF),
            pltpu.VMEM((D, F), BF),
            pltpu.VMEM((D, F), BF),
            pltpu.VMEM((F, D), BF),
            pltpu.VMEM((D + 2 * Dh, D), BF),
            pltpu.VMEM((NB * H, Dh, TQ), BF),
            pltpu.VMEM((NB * H, Dh, TQ), F32),
            pltpu.VMEM((S, Dh), BF),
            pltpu.VMEM((Dh, S), BF),
            pltpu.VMEM((Dh, NKB, 128), F32),
            pltpu.VMEM((G, S, TQ), F32),
            pltpu.VMEM((G, S, TQ), F32),
            pltpu.VMEM((G, 1, TQ), F32),
            pltpu.VMEM((D, TQ), F32),
            pltpu.VMEM((G, 8, TQ), F32),
            pltpu.SemaphoreType.DMA((1 + NB + 4,)),
        ],
        compiler_params=pltpu.CompilerParams(
            dimension_semantics=("arbitrary",),
            vmem_limit_bytes=100 * 1024 * 1024,
        ),
    )(A_wk.T, A_wv.T, gate_w, A_x.reshape(S, D), A_wq, A_wo, B_w_gate, B_w_up, B_w_down)
    return out.reshape(B, S, D)
```
